```python
import os as _os
_os.environ.setdefault("JAX_PLATFORMS", "cpu")
import jax
import jax.numpy as jnp

def _softmax(x, axis=-1):
    return jax.nn.softmax(x, axis=axis)
def _gelu(x):
    return jax.nn.gelu(x, approximate=True)
def _silu(x):
    return jax.nn.silu(x)
def _sigmoid(x):
    return jax.nn.sigmoid(x)
def _layernorm(x, axis=-1, eps=1e-5):
    m = jnp.mean(x, axis=axis, keepdims=True)
    v = jnp.var(x, axis=axis, keepdims=True)
    return (x - m) / jnp.sqrt(v + eps)
def _scatter_add(tgt, idx, src, axis=0):
    return tgt.at[idx].add(src)
def _segment_sum(src, seg, n):
    return jax.ops.segment_sum(src, seg, n)
class _Rng:
    def __init__(self, key):
        self._k = key
    def _next(self):
        self._k, sub = jax.random.split(self._k)
        return sub
    def normal(self, shape):
        return jax.random.normal(self._next(), shape, dtype=jnp.bfloat16)
    def randint(self, lo, hi, shape):
        return jax.random.randint(self._next(), shape, lo, hi, dtype=jnp.int32)
    def uniform(self, shape, lo=0.0, hi=1.0):
        return jax.random.uniform(self._next(), shape, jnp.bfloat16, lo, hi)
    def permutation(self, n):
        return jax.random.permutation(self._next(), n)


kernel_name = 'sequential_preLN__softmax_full_mha__swiglu_ffn__prompt'

def setup_inputs():
    _rng = _Rng(jax.random.key(int.from_bytes(__import__("os").urandom(4), "little")))
    _w = (lambda a: (lambda t: t.astype(jnp.bfloat16) if jnp.issubdtype(t.dtype, jnp.floating) else t)(jnp.asarray(a)))
    def _A_setup():
        B, S, D = 1, 2048, 512
        return {
            "x": _w((lambda *s: _rng.normal(s) * 0.05)(B, S, D)),
            "wqkv": _w((lambda *s: _rng.normal(s) * 0.05)(D, 3 * D)),
            "wo": _w((lambda *s: _rng.normal(s) * 0.05)(D, D)),
        }
    _A_in = _A_setup()

    def _B_setup():
        B, S, D, F = 1, 2048, 512, 1792
        return {
            "x": _w((lambda *s: _rng.normal(s) * 0.05)(B, S, D)),
            "w_gate": _w((lambda *s: _rng.normal(s) * 0.05)(D, F)),
            "w_up": _w((lambda *s: _rng.normal(s) * 0.05)(D, F)),
            "w_down": _w((lambda *s: _rng.normal(s) * 0.05)(F, D)),
        }
    _B_in = _B_setup()

    return {
        "A_x": _A_in["x"],
        "A_wqkv": _A_in["wqkv"],
        "A_wo": _A_in["wo"],
        "B_x": _B_in["x"],
        "B_w_gate": _B_in["w_gate"],
        "B_w_up": _B_in["w_up"],
        "B_w_down": _B_in["w_down"],
    }

def reference(A_x, A_wqkv, A_wo, B_x, B_w_gate, B_w_up, B_w_down):
    def _A_ref(x, wqkv, wo):
        B, S, D = x.shape
        H = 32; Dh = D // H
        qkv = (lambda x, *d: x.transpose(*d))((x @ wqkv).reshape(B, S, 3, H, Dh), 2, 0, 3, 1, 4)
        q, k, v = qkv[0], qkv[1], qkv[2]
        scale = Dh ** -0.5
        scores = jnp.einsum("bhqd,bhkd->bhqk", q, k) * scale
        p = _softmax(scores, axis=-1)
        o = jnp.einsum("bhqk,bhkd->bhqd", p, v)
        return (lambda x, *d: x.transpose(*d))(o, 0, 2, 1, 3).reshape(B, S, D) @ wo

    def _B_ref(x, w_gate, w_up, w_down):
        g = _silu(x @ w_gate)
        u = x @ w_up
        return (g * u) @ w_down

    x = A_x
    h = x + _A_ref(_layernorm(x, axis=-1), A_wqkv, A_wo)
    h2 = h + _B_ref(_layernorm(h, axis=-1), B_w_gate, B_w_up, B_w_down)
    return h2
```

```python
import numpy as np
import jax
import jax.numpy as jnp
from jax import lax
import jax.experimental.pallas as pl
import jax.experimental.pallas.tpu as pltpu

F32, BF16, U32 = jnp.float32, jnp.bfloat16, jnp.uint32
H = 32
LN_EPS = 1e-5
LANES = 128
BQ = 512
KT = 128
VR = 16
LAG = 2
RC = 256
MXU_ONLY = (0, -1)
L_LO, L_HI, V_HI = 2.0 ** -40, 2.0 ** 40, 2.0 ** 80


def _layernorm(x):
    m = jnp.mean(x, axis=-1, keepdims=True)
    c = x - m
    v = jnp.mean(c * c, axis=-1, keepdims=True)
    return c * lax.rsqrt(v + LN_EPS)


def _silu(g):
    half = 0.5 * g
    return half + half * jnp.tanh(half)


def _fold8(p):
    return jnp.sum(p.reshape(-1, 8, p.shape[-1]), axis=0)


def _words(x):
    return pltpu.bitcast(x.astype(BF16), U32)


def _bf(words):
    return pltpu.bitcast(words, BF16)


def _dot(a, b, contract=(1, 0)):
    return lax.dot_general(a, b, (((contract[0],), (contract[1],)), ((), ())),
                           preferred_element_type=F32)


def _quads(a):
    r, c = a.shape[0] // 2, a.shape[1] // 2
    return a[:r, :c], a[:r, c:], a[r:, :c], a[r:, c:]


def _blocks(c11, c12, c21, c22):
    return jnp.concatenate([jnp.concatenate([c11, c12], axis=1),
                            jnp.concatenate([c21, c22], axis=1)], axis=0)


def _strassen_lhs(a11, a12, a21, a22):
    return [a11 + a22, a21 + a22, a11, a22, a11 + a12, a21 - a11, a12 - a22]


def _strassen_rhs(b11, b12, b21, b22):
    return [b11 + b22, b11, b12 - b22, b21 - b11, b22, b11 + b12, b21 + b22]


def _strassen_out(m):
    return (m[0] + m[3] - m[4] + m[6], m[2] + m[4], m[1] + m[3], m[0] - m[1] + m[2] + m[5])


PLAIN = {1: 0, 4: 1}


def _store_rhs(sums, index, quads):
    for i, b in enumerate(_strassen_rhs(*quads)):
        if i not in PLAIN:
            sums[(i,) + index] = b.astype(BF16)


def _rhs(i, sums, whole, c0, n):
    if i not in PLAIN:
        return sums[:, c0:c0 + n]
    r, c = whole.shape[0] // 2, whole.shape[1] // 2
    r0, c0 = PLAIN[i] * r, PLAIN[i] * c + c0
    return whole[r0:r0 + r, c0:c0 + n]


def _kernel(x_hbm, wqkv_hbm, wo_hbm, wg_hbm, wu_hbm, wd_hbm, out_hbm,
            x_v, wqkv_v, wo_v, wgu_v, wd_v, sk_v, sqv_v, sgu_v, sd_v,
            k_v, q_v, q32_v, v_v, s0_v, o_v, h_v, hs_v, a_v, out_v, in_sem, out_sem):
    S, D = x_v.shape
    F = wd_v.shape[0]
    dh = D // H
    nq, nk, nr = S // BQ, S // KT, S // RC

    def chunk(r, n=RC):
        return pl.ds(pl.multiple_of(r * n, n), n)

    def x_copy(r):
        return pltpu.make_async_copy(x_hbm.at[chunk(r)], x_v.at[chunk(r)], in_sem.at[r])

    def qkv_copy(i):
        return pltpu.make_async_copy(wqkv_hbm.at[:, pl.ds(i * D, D)], wqkv_v.at[i],
                                     in_sem.at[nr + i])

    def out_copy(r):
        return pltpu.make_async_copy(out_v.at[chunk(r)], out_hbm.at[chunk(r)], out_sem.at[r])

    w_cp = [pltpu.make_async_copy(s, d, in_sem.at[nr + 3 + i]) for i, (s, d) in enumerate(
        [(wg_hbm, wgu_v.at[0]), (wu_hbm, wgu_v.at[1]), (wd_hbm, wd_v), (wo_hbm, wo_v)])]
    for c in (x_copy(0), qkv_copy(0), qkv_copy(2), qkv_copy(1), x_copy(1), x_copy(2)):
        c.start()

    qscale = float(dh ** -0.5 * np.log2(np.e))
    wk_v = wqkv_v.at[1]

    def store_lhs(slot, a):
        for i, t in enumerate(_strassen_lhs(*_quads(a))):
            hs_v[slot, i] = t.astype(BF16)

    def normalize(r, slot):
        store_lhs(slot, _layernorm(x_v[chunk(r), :].astype(F32)))

    def qkv(r, slot, v_max):
        normalize(jnp.minimum(r + 1, nr - 1), 1 - slot)
        xs = [hs_v[slot, i] for i in range(7)]

        def transposed(w):
            c11, c12, c21, c22 = _strassen_out([_dot(sqv_v[w, i], xs[i], (1, 1)) for i in range(7)])
            return _blocks(c11, c21, c12, c22)

        k = _words(_blocks(*_strassen_out(
            [_dot(xs[i], _rhs(i, sk_v.at[i], wk_v, 0, D // 2)) for i in range(7)])))
        for h in range(H):
            k_v[h, chunk(r, RC // 2), :] = k[:, h * dh:(h + 1) * dh]
        q = transposed(0) * qscale
        q32_v[:, :, chunk(r)] = q.reshape(H, dh, RC)
        q_v[:, :, chunk(r)] = _words(q).reshape(H, dh // 2, RC)
        v = transposed(1)
        v_v[:, :, chunk(r)] = _words(v).reshape(H, dh // 2, RC)
        m = jnp.max(jnp.abs(v).reshape(D // 8, 8, RC), axis=0)
        for t in range(0, RC, LANES):
            v_max = jnp.maximum(v_max, m[:, t:t + LANES])
        return v_max

    def qkv_pair(i, v_max):
        x_copy(2 * i + 1).wait()

        @pl.when(2 * i + 2 < nr)
        def _():
            x_copy(2 * i + 2).wait()
        return qkv(2 * i + 1, 1, qkv(2 * i, 0, v_max))

    x_copy(0).wait()
    normalize(0, 0)
    for w, part in enumerate((0, 2)):
        qkv_copy(part).wait()
        c11, c21, c12, c22 = _quads(wqkv_v[part].T.astype(F32))
        for i, b in enumerate(_strassen_rhs(c11, c12, c21, c22)):
            sqv_v[w, i] = b.astype(BF16)
    qkv_copy(1).wait()
    for c in [x_copy(r) for r in range(3, nr)] + w_cp:
        c.start()
    _store_rhs(sk_v, (), _quads(wk_v[...].astype(F32)))
    v_max = lax.fori_loop(0, nr // 2, qkv_pair, jnp.zeros((8, LANES), F32))
    for c in w_cp:
        c.wait()

    items = [(u, c) for u in range(nq) for c in range(nk)]
    vpu_rows = [0 if n in MXU_ONLY or n - len(items) in MXU_ONLY else VR
                for n in range(len(items))]

    def key_words(h, n):
        c = items[n][1]
        return k_v[h, c * KT // 2:((c + 1) * KT - vpu_rows[n]) // 2, :]

    def first_scores(h):
        s0_v[...] = _dot(_bf(key_words(h, 0)), _bf(q_v[h, :, 0:BQ]))

    def spread_keys(h, c):
        kw = k_v[h, ((c + 1) * KT - VR) // 2:(c + 1) * KT // 2, :]
        return [_bf(jnp.broadcast_to(kw[:, d:d + 1], (VR // 2, LANES))).astype(F32)
                for d in range(dh)]

    def vpu_scores(h, u, kb):
        part, marks = [None] * (BQ // LANES), []
        step = dh // (2 * len(part))
        for d in range(dh):
            for i in range(len(part)):
                t = u * BQ + i * LANES
                prod = kb[d] * q32_v[h, d:d + 1, t:t + LANES]
                part[i] = prod if d == 0 else part[i] + prod
            if d % step == step - 1:
                j = d // step
                marks.append(part[j // 2][8 * (j % 2):8 * (j % 2) + 8])
        return jnp.concatenate(part, axis=1), marks

    def prepare_ffn_weights(h):
        rb = D // H
        w, g = h // (H // 2), h % (H // 2)
        top = wgu_v[w, chunk(g, rb), :].astype(F32)
        bot = wgu_v[w, chunk(g + H // 2, rb), :].astype(F32)
        _store_rhs(sgu_v, (w, chunk(g, rb)), _quads(jnp.concatenate([top, bot], axis=0)))
        rb = 16 * pl.cdiv(F // 2, 16 * H)
        g = jnp.minimum(h, F // 2 // rb - 1)
        top = wd_v[chunk(g, rb), :].astype(F32)
        bot = wd_v[chunk(g + F // 2 // rb, rb), :].astype(F32)
        _store_rhs(sd_v, (chunk(g, rb),), _quads(jnp.concatenate([top, bot], axis=0)))

    def head(h, span):
        lo, hi = span
        s_mxu, s_vpu, marks, spread = {}, {}, {}, {}
        keep = jnp.full((8, dh), h // 1000, jnp.int32) == 0
        for n in range(len(items) + LAG):
            if 0 <= n - 1 < len(items) and vpu_rows[n - 1]:
                u, c = items[n - 1]
                if c not in spread:
                    spread[c] = spread_keys(h, c)
                s_vpu[n - 1], marks[n - 1] = vpu_scores(h, u, spread[c])
            if n == 0:
                s_mxu[n] = s0_v[...]
            elif n < len(items):
                u, kw = items[n][0], key_words(h, n)
                if n - 1 in marks:
                    m = kw.shape[0] // 8
                    kw = jnp.concatenate(
                        [jnp.where(keep, kw[8 * j:8 * j + 8], pltpu.bitcast(t, U32)[:, :dh])
                         for j, t in enumerate(marks[n - 1][-m:])], axis=0)
                s_mxu[n] = _dot(_bf(kw), _bf(q_v[h, :, u * BQ:(u + 1) * BQ]))
            elif n == len(items):
                first_scores(jnp.minimum(h + 1, H - 1))
            if n >= LAG:
                u, c = items[n - LAG]
                s = s_mxu.pop(n - LAG)
                if vpu_rows[n - LAG]:
                    s = jnp.concatenate([s, s_vpu.pop(n - LAG)], axis=0)
                p = jnp.exp2(s)
                total = _fold8(p) if c == 0 else total + _fold8(p)
                pv = _dot(_bf(v_v[h, :, c * KT:(c + 1) * KT]), p.astype(BF16))
                acc = pv if c == 0 else acc + pv
                if c == nk - 1:
                    tot = jnp.broadcast_to(jnp.sum(total, axis=0, keepdims=True), (8, BQ))
                    inv = jnp.concatenate([1.0 / tot] * (dh // 8), axis=0)
                    o_v[h, :, u * BQ:(u + 1) * BQ] = (acc * inv).astype(BF16)
                    for t in range(0, BQ, LANES):
                        lo = jnp.minimum(lo, tot[:, t:t + LANES])
                        hi = jnp.maximum(hi, tot[:, t:t + LANES])
        prepare_ffn_weights(h)
        return lo, hi

    first_scores(0)
    lo, hi = lax.fori_loop(0, H, head, (jnp.ones((8, LANES), F32),) * 2)
    safe = (lo >= L_LO) & (hi <= L_HI) & (v_max <= V_HI)

    @pl.when(jnp.max(jnp.where(safe, 0.0, 1.0)) > 0.0)
    def _():
        def redo(i, carry):
            h, cols = i // nq, chunk(i % nq, BQ)
            s = _dot(_bf(k_v[h]), _bf(q_v[h, :, cols]))
            p = jnp.exp2(s - jnp.max(s, axis=0, keepdims=True))
            p = p / jnp.sum(p, axis=0, keepdims=True)
            o_v[h, :, cols] = _dot(_bf(v_v[h]), p.astype(BF16)).astype(BF16)
            return carry
        lax.fori_loop(0, H * nq, redo, 0)

    def project(r, slot):
        attn = _dot(o_v[:, :, chunk(r)].reshape(D, RC), wo_v[...], (0, 0))
        res = x_v[chunk(r), :].astype(F32) + attn
        h_v[slot] = res
        store_lhs(slot, _layernorm(res))

    def ffn(r, carry):
        slot = r % 2
        for f in range(0, F // 2, LANES):
            m = [_dot(hs_v[slot, i], jnp.concatenate(
                [_rhs(i, sgu_v.at[i, w], wgu_v.at[w], f, LANES) for w in range(2)], axis=1))
                 for i in range(7)]
            act = [_silu(c[:, :LANES]) * c[:, LANES:] for c in _strassen_out(m)]
            for i, a in enumerate(_strassen_lhs(*act)):
                a_v[i, :, f:f + LANES] = a.astype(BF16)
        project(jnp.minimum(r + 1, nr - 1), 1 - slot)
        y = h_v[slot] + _blocks(*_strassen_out(
            [_dot(a_v[i], _rhs(i, sd_v.at[i], wd_v, 0, D // 2)) for i in range(7)]))
        out_v[chunk(r), :] = y.astype(out_v.dtype)
        out_copy(r).start()
        return carry

    project(0, 0)
    lax.fori_loop(0, nr, ffn, 0)
    for r in range(nr):
        out_copy(r).wait()


@jax.jit
def pallas_sequential_preLN__softmax_full_mha__swiglu_ffn__prompt_kernel(
    A_x: jax.Array,
    A_wqkv: jax.Array,
    A_wo: jax.Array,
    B_x: jax.Array,
    B_w_gate: jax.Array,
    B_w_up: jax.Array,
    B_w_down: jax.Array,
):
    del B_x
    B, S, D = A_x.shape
    F = B_w_gate.shape[1]
    dh = D // H
    assert B == 1 and S % (2 * RC) == 0 and S % BQ == 0 and F % (2 * LANES) == 0
    vm = pltpu.VMEM
    out = pl.pallas_call(
        _kernel,
        in_specs=[pl.BlockSpec(memory_space=pl.ANY)] * 6,
        out_specs=pl.BlockSpec(memory_space=pl.ANY),
        out_shape=jax.ShapeDtypeStruct((S, D), A_x.dtype),
        scratch_shapes=[
            vm((S, D), A_x.dtype), vm((3, D, D), BF16), vm((D, D), BF16),
            vm((2, D, F), BF16), vm((F, D), BF16),
            vm((7, D // 2, D // 2), BF16), vm((2, 7, D // 2, D // 2), BF16),
            vm((7, 2, D // 2, F // 2), BF16), vm((7, F // 2, D // 2), BF16),
            vm((H, S // 2, dh), U32),
            vm((H, dh // 2, S), U32), vm((H, dh, S), F32),
            vm((H, dh // 2, S), U32),
            vm((KT, BQ), F32),
            vm((H, dh, S), BF16),
            vm((2, RC, D), F32), vm((2, 7, RC // 2, D // 2), BF16), vm((7, RC // 2, F // 2), BF16),
            vm((S, D), A_x.dtype),
            pltpu.SemaphoreType.DMA((S // RC + 7,)),
            pltpu.SemaphoreType.DMA((S // RC,)),
        ],
        compiler_params=pltpu.CompilerParams(vmem_limit_bytes=100 * 2 ** 20),
        name="preln_mha_swiglu",
    )(A_x.reshape(S, D), A_wqkv, A_wo, B_w_gate, B_w_up, B_w_down)
    return out.reshape(B, S, D)
```
